```python
import os as _os
_os.environ.setdefault('JAX_PLATFORMS', 'cpu')
import jax
import jax.numpy as jnp

def _softmax(x, axis=-1):
    return jax.nn.softmax(x, axis=axis)

def _gelu(x):
    return jax.nn.gelu(x, approximate=True)

def _silu(x):
    return jax.nn.silu(x)

def _sigmoid(x):
    return jax.nn.sigmoid(x)

def _layernorm(x, axis=-1, eps=1e-05):
    m = jnp.mean(x, axis=axis, keepdims=True)
    v = jnp.var(x, axis=axis, keepdims=True)
    return (x - m) / jnp.sqrt(v + eps)

def _scatter_add(tgt, idx, src, axis=0):
    return tgt.at[idx].add(src)

def _segment_sum(src, seg, n):
    return jax.ops.segment_sum(src, seg, n)

class _Rng:

    def __init__(self, key):
        self._k = key

    def _next(self):
        self._k, sub = jax.random.split(self._k)
        return sub

    def normal(self, shape):
        return jax.random.normal(self._next(), shape, dtype=jnp.bfloat16)

    def randint(self, lo, hi, shape):
        return jax.random.randint(self._next(), shape, lo, hi, dtype=jnp.int32)

    def uniform(self, shape, lo=0.0, hi=1.0):
        return jax.random.uniform(self._next(), shape, jnp.bfloat16, lo, hi)

    def permutation(self, n):
        return jax.random.permutation(self._next(), n)
kernel_name = 'standalone__conformer_family_e_branchformer__speech'

def setup_inputs():
    _rng = _Rng(jax.random.key(int.from_bytes(__import__("os").urandom(4), "little")))
    _w = lambda a: (lambda t: t.astype(jnp.bfloat16) if jnp.issubdtype(t.dtype, jnp.floating) else t)(jnp.asarray(a))
    B, T, D, K = (2, 4000, 256, 31)
    return {'x': _w((lambda *s: _rng.normal(s) * 0.05)(B, T, D)), 'w_qkv': _w((lambda *s: _rng.normal(s) * 0.05)(D, 3 * D)), 'w_att_out': _w((lambda *s: _rng.normal(s) * 0.05)(D, D)), 'w_mlp_in': _w((lambda *s: _rng.normal(s) * 0.05)(D, 2 * D)), 'dw_csgu': _w((lambda *s: _rng.normal(s) * 0.05)(K, D)), 'w_mlp_out': _w((lambda *s: _rng.normal(s) * 0.05)(D, D)), 'dw_merge': _w((lambda *s: _rng.normal(s) * 0.05)(K, 2 * D)), 'w_merge': _w((lambda *s: _rng.normal(s) * 0.05)(2 * D, D))}

def reference(x, w_qkv, w_att_out, w_mlp_in, dw_csgu, w_mlp_out, dw_merge, w_merge):
    B, T, D = x.shape
    K = dw_csgu.shape[0]
    pad = K // 2
    xa = _layernorm(x, axis=-1)
    qkv = jnp.einsum('btd,de->bte', xa, w_qkv)
    q, k, v = (qkv[..., :D].copy(), qkv[..., D:2 * D].copy(), qkv[..., 2 * D:].copy())
    scores = jnp.einsum('btd,bsd->bts', q, k) * D ** (-0.5)
    p = _softmax(scores, axis=-1)
    attn = jnp.einsum('bts,bsd->btd', p, v)
    glob = jnp.einsum('btd,de->bte', attn, w_att_out)
    xc = _layernorm(x, axis=-1)
    h = _gelu(jnp.einsum('btd,de->bte', xc, w_mlp_in))
    u, g = (h[..., :D].copy(), h[..., D:].copy())
    g = _layernorm(g, axis=-1)
    gp = jnp.pad(g, ((0, 0), (pad, pad), (0, 0)))
    gc = jnp.zeros_like(g)
    for i in range(K):
        gc = gc + gp[:, i:i + T, :] * dw_csgu[i][None, None, :]
    loc = jnp.einsum('btd,de->bte', u * gc, w_mlp_out)
    m = jnp.concatenate([glob, loc], axis=-1)
    mp = jnp.pad(m, ((0, 0), (pad, pad), (0, 0)))
    mc = jnp.zeros_like(m)
    for i in range(K):
        mc = mc + mp[:, i:i + T, :] * dw_merge[i][None, None, :]
    m = m + mc
    return x + jnp.einsum('btc,cd->btd', m, w_merge)
```

```python
import functools
import math

import jax
import jax.numpy as jnp
import jax.experimental.pallas as pl
import jax.experimental.pallas.tpu as pltpu

_NT = (((1,), (1,)), ((), ()))
_F32 = jnp.float32
_BF16 = jnp.bfloat16


def _make_kernel(B, T, D, K, M, NC, RB, PR, HK, DBG, ORD, AO, AR):
    TP = -(-T // 128) * 128
    CK = TP // NC
    PAD = K // 2
    H = 16
    R = T + 2 * H
    M2 = 2 * M
    NS = D // 128
    NPB = T // M2
    NPAIR = B * NPB
    NP = M // PR
    QS = -(-M // 64) * 64
    eps = 1e-5
    TAPS = [k for b in range(8) for k in range(b, K, 8)]
    qscale = (D ** -0.5) * math.log2(math.e)

    GC1 = math.sqrt(2.0 / math.pi)
    GC2 = GC1 * 0.044715

    def ln(v, eps=eps):
        mu = jnp.mean(v, axis=-1, keepdims=True)
        c = v - mu
        var = jnp.mean(c * c, axis=-1, keepdims=True)
        return c * jax.lax.rsqrt(var + eps)

    def kernel(x_hbm, wqkv_ref, wo_ref, wmi_ref, dwc_ref, wmo_ref, dwm_ref, wmg_ref, out_hbm,
               x_v, o_v, wall, wbc, wbm, k_s, q_s, v_s, u_s, g_s, mg_s, ml_s, zero_s, xsem, osem):
        zero_s[0] = 0

        def x_copy(t):
            return pltpu.make_async_copy(x_hbm.at[t], x_v.at[t], xsem.at[t])

        def o_copy(p):
            return pltpu.make_async_copy(o_v.at[p], out_hbm.at[p], osem.at[p])

        for t in range(NPAIR):
            x_copy(t).start()

        wq = wqkv_ref[:, 0:D]
        wk = wqkv_ref[:, D:2 * D]
        wv = wqkv_ref[:, 2 * D:3 * D]
        a = jax.lax.dot_general(wq, wk, _NT, preferred_element_type=_F32) * qscale
        wvo = jnp.dot(wv, wo_ref[...], preferred_element_type=_F32)
        col = {n: slice(i * D, (i + 1) * D) for i, n in enumerate(ORD)}
        wall[:, col['u']] = wmi_ref[:, 0:D]
        wall[:, col['g']] = wmi_ref[:, D:2 * D]
        wall[:, col['q']] = a.astype(_BF16)
        wall[:, col['v']] = wvo.astype(_BF16)
        dwc = dwc_ref[...].astype(_F32) * 0.5
        dwm = dwm_ref[...].astype(_F32)
        for k in range(K):
            for s in range(NS):
                wbc[s, k] = jnp.broadcast_to(dwc[k:k + 1, s * 128:(s + 1) * 128], (8, 128))
            for s in range(2 * NS):
                w = dwm[k:k + 1, s * 128:(s + 1) * 128]
                if k == PAD:
                    w = w + 1.0
                wbm[s, k] = jnp.broadcast_to(w, (8, 128))
        zf = jnp.zeros((H, 128), _F32)
        for b in range(B):
            for s in range(NS):
                for m_s in (g_s, mg_s, ml_s):
                    m_s[s, b * R:b * R + H, :] = zf
                    m_s[s, b * R + H + T:(b + 1) * R, :] = zf
                if TP > T:
                    k_s[b, s, T:TP, :] = jnp.zeros((TP - T, 128), _BF16)
                    v_s[b, s, T:TP, :] = jnp.zeros((TP - T, 128), _BF16)

        zi = jnp.zeros((PR + 2 * H, 128), _F32)
        for s in range(NS):
            mg_s[s, M2 - PR:M2 + 2 * H, :] = zi
            ml_s[s, M2 - PR:M2 + 2 * H, :] = zi

        def fresh(p):
            return p + zero_s[0]

        def cbase(p):
            b = p // NPB
            return pl.multiple_of(b * R + (p - b * NPB) * M2, 32)

        def batch_of(p):
            b = 0
            for j in range(1, B):
                b = b + (p >= j * NPB).astype(jnp.int32)
            return b

        def krow_of(t):
            b = batch_of(t)
            return b, pl.multiple_of((t - b * NPB) * M2, 16)

        def a1(t):
            b, krow = krow_of(t)
            xa = ln(x_v[t].astype(_F32))
            for s in range(NS):
                k_s[b, s, pl.ds(krow, M2), :] = xa[:, s * 128:(s + 1) * 128].astype(_BF16)

        def a2(t, nxt):
            b, krow = krow_of(t)
            crow = cbase(t)
            xa = jnp.concatenate([k_s[b, s, pl.ds(krow, M2), :] for s in range(NS)], axis=1)
            if nxt is not None and AO == 0:
                a1(nxt)
            y = jnp.dot(xa, wall[...], preferred_element_type=_F32)
            gelu2 = lambda hx: hx * (1.0 + jnp.tanh(hx * (GC1 + GC2 * (hx * hx))))
            u_s[t] = gelu2(y[:, col['u']])
            g = ln(gelu2(y[:, col['g']]), 4.0 * eps)
            q = y[:, col['q']]
            v = y[:, col['v']]
            for s in range(NS):
                g_s[s, pl.ds(crow + H, M2), :] = g[:, s * 128:(s + 1) * 128]
                for j in range(2):
                    q_s[t, j, s, 0:M, :] = q[j * M:(j + 1) * M, s * 128:(s + 1) * 128].astype(_BF16)
                v_s[b, s, pl.ds(krow, M2), :] = v[:, s * 128:(s + 1) * 128].astype(_BF16)
            if nxt is not None and AO == 1:
                a1(nxt)

        def phase_a(t, carry):
            x_copy(t + 1).wait()
            a2(t, jax.lax.rem(t + 1, NPAIR) if AR else t + 1)
            return carry

        x_copy(0).wait()
        a1(fresh(0))
        jax.lax.fori_loop(0, NPAIR - 1, phase_a, 0)
        a2(fresh(NPAIR - 1), None)

        def conv(src, wb, s, base, off, nrows, ws=0):
            outs = []
            for r in range(nrows // RB):
                acc = None
                for k in TAPS:
                    xk = src[s, pl.ds(base + (off + H + r * RB + k - PAD), RB), :].reshape(RB // 8, 8, 128)
                    term = xk * wb[ws + s, k][None]
                    acc = term if acc is None else acc + term
                outs.append(acc.reshape(RB, 128))
            return jnp.concatenate(outs, axis=0) if len(outs) > 1 else outs[0]

        def att(p, j, hooks):
            crow = cbase(p)
            b = batch_of(p)
            pq = jax.lax.rem(p, NPAIR)
            q = jnp.concatenate([q_s[pq, j, s, 0:M, :] for s in range(NS)], axis=1)

            def kv(ref, c):
                return jnp.concatenate([ref[b, s, c * CK:(c + 1) * CK, :] for s in range(NS)], axis=1)

            def qk(c):
                s = jax.lax.dot_general(q, kv(k_s, c), _NT, preferred_element_type=_F32)
                if c == NC - 1 and TP > T:
                    lane = jax.lax.broadcasted_iota(jnp.int32, (M, 128), 1)
                    s_last = jnp.where(lane < T - (TP - 128), s[:, CK - 128:], -jnp.inf)
                    s = jnp.concatenate([s[:, :CK - 128], s_last], axis=1)
                return s

            s_next = qk(0)
            for c in range(NC):
                s = s_next
                if c + 1 < NC:
                    s_next = qk(c + 1)
                m_c = jnp.max(s, axis=1, keepdims=True)
                if c == 0:
                    m_new = m_c
                else:
                    m_new = jnp.maximum(m_run, m_c)
                    alpha = jnp.exp2(m_run - m_new)
                pr = jnp.exp2(s - m_new)
                l_c = pr[:, 0:128]
                for jj in range(1, CK // 128):
                    l_c = l_c + pr[:, jj * 128:(jj + 1) * 128]
                pv = jnp.dot(pr.astype(_BF16), kv(v_s, c), preferred_element_type=_F32)
                if c == 0:
                    l = l_c
                    acc = pv
                else:
                    l = l * alpha + l_c
                    acc = acc * alpha + pv
                m_run = m_new
                for hk in hooks.get(c, []):
                    hk()
            lsum = jnp.sum(l, axis=1, keepdims=True)
            glob = acc * (1.0 / lsum)
            for s in range(NS):
                mg_s[s, pl.ds(crow + (H + j * M), M), :] = glob[:, s * 128:(s + 1) * 128]

        def loc_piece(p, o):
            def h():
                crow = cbase(p)
                gc = jnp.concatenate([conv(g_s, wbc, s, crow, o, PR) for s in range(NS)], axis=1)
                z = (u_s[p, o:o + PR, :] * gc).astype(_BF16)
                y = jnp.dot(z, wmo_ref[...], preferred_element_type=_F32)
                for s in range(NS):
                    ml_s[s, pl.ds(crow + (H + o), PR), :] = y[:, s * 128:(s + 1) * 128]
            return h

        def merge_pieces(p, o):
            st = []

            def h1():
                mloc = jnp.concatenate([conv(ml_s, wbm, s, cbase(p), o, PR, NS) for s in range(NS)], axis=1).astype(_BF16)
                st.append(x_v[p, o:o + PR, :].astype(_F32) + jnp.dot(mloc, wmg_ref[D:2 * D, :], preferred_element_type=_F32))

            def h2():
                mglob = jnp.concatenate([conv(mg_s, wbm, s, cbase(p), o, PR) for s in range(NS)], axis=1).astype(_BF16)
                y = st[0] + jnp.dot(mglob, wmg_ref[0:D, :], preferred_element_type=_F32)
                o_v[p, o:o + PR, :] = y.astype(_BF16)
            return [h1, h2]

        def body(p, j, merges):
            pieces = []
            for (pp, o) in merges:
                pieces += merge_pieces(pp, o)
            pieces += [loc_piece(p, j * M + r * PR) for r in range(NP)]
            hooks = {}
            for i, pc in enumerate(pieces):
                c = HK[i] if len(pieces) == len(HK) else 1 + (i * (NC - 3)) // len(pieces)
                hooks.setdefault(c, []).append(pc)
            att(p, j, hooks)

        def even(p):
            body(p, 0, [(p - 1, M - PR + r * PR) for r in range(NP)])

        def odd(p, pprev, oprev):
            body(p, 1, [(pprev, oprev)] + [(p, r * PR) for r in range(NP - 1)])

        def pair(p, carry):
            @pl.when(p > 0)
            def _():
                even(fresh(p))

            @pl.when(p == 0)
            def _():
                body(fresh(p), 0, [])

            p2 = fresh(p)
            odd(p2, jnp.maximum(p2 - 1, 0), M2 - PR)

            @pl.when(p > 0)
            def _():
                o_copy(p - 1).start()
            return carry

        if not (DBG & 1):
            jax.lax.fori_loop(0, NPAIR, pair, 0)
        else:
            def fake(p, c):
                z = (u_s[p, 0:16, 0:128] + g_s[0, pl.ds(p * 16, 16), :] + q_s[p, 0, 0, 0:16, :].astype(_F32)
                     + k_s[0, 0, pl.ds(p * 16, 16), :].astype(_F32) + v_s[0, 0, pl.ds(p * 16, 16), :].astype(_F32))
                o_v[p, 0:16, 0:128] = z.astype(_BF16)
                return c
            jax.lax.fori_loop(0, NPAIR, fake, 0)
            for n in range(NPAIR - 1):
                o_copy(n).start()
        pl_ = fresh(NPAIR - 1)
        for r in range(NP + 1):
            for h in merge_pieces(pl_, M - PR + r * PR):
                h()
        o_copy(NPAIR - 1).start()
        for n in range(NPAIR):
            o_copy(n).wait()

    scratch = [
        pltpu.VMEM((NPAIR, M2, D), _BF16),
        pltpu.VMEM((NPAIR, M2, D), _BF16),
        pltpu.VMEM((D, 4 * D), _BF16),
        pltpu.VMEM((NS, 32, 8, 128), _F32),
        pltpu.VMEM((2 * NS, 32, 8, 128), _F32),
        pltpu.VMEM((B, NS, TP, 128), _BF16),
        pltpu.VMEM((NPAIR, 2, NS, QS, 128), _BF16),
        pltpu.VMEM((B, NS, TP, 128), _BF16),
        pltpu.VMEM((NPAIR, M2, D), _F32),
        pltpu.VMEM((NS, B * R, 128), _F32),
        pltpu.VMEM((NS, B * R, 128), _F32),
        pltpu.VMEM((NS, B * R, 128), _F32),
        pltpu.SMEM((1,), jnp.int32),
        pltpu.SemaphoreType.DMA((NPAIR,)),
        pltpu.SemaphoreType.DMA((NPAIR,)),
    ]
    return kernel, scratch, NPAIR, M2


def build(M=400, NC=16, RB=80, PR=80, HK=(1, 2, 3, 4, 4, 5, 6, 7, 7, 8, 9, 10, 10, 11, 12), DBG=0, ORD='qguv', AO=0, AR=0):
    @jax.jit
    def fn(x, w_qkv, w_att_out, w_mlp_in, dw_csgu, w_mlp_out, dw_merge, w_merge):
        B, T, D = x.shape
        K = dw_csgu.shape[0]
        kernel, scratch, NPAIR, M2 = _make_kernel(B, T, D, K, M, NC, RB, PR, HK, DBG, ORD, AO, AR)
        vm = pl.BlockSpec(memory_space=pltpu.VMEM)
        out = pl.pallas_call(
            kernel,
            out_shape=jax.ShapeDtypeStruct((NPAIR, M2, D), x.dtype),
            in_specs=[pl.BlockSpec(memory_space=pl.ANY)] + [vm] * 7,
            out_specs=pl.BlockSpec(memory_space=pl.ANY),
            scratch_shapes=scratch,
            compiler_params=pltpu.CompilerParams(vmem_limit_bytes=110 * 1024 * 1024),
        )(x.reshape(NPAIR, M2, D), w_qkv, w_att_out, w_mlp_in, dw_csgu, w_mlp_out, dw_merge, w_merge)
        return out.reshape(B, T, D)
    return fn


_impl = build(**OPQ)


@jax.jit
def pallas_standalone__conformer_family_e_branchformer__speech_kernel(
    x: jax.Array,
    w_qkv: jax.Array,
    w_att_out: jax.Array,
    w_mlp_in: jax.Array,
    dw_csgu: jax.Array,
    w_mlp_out: jax.Array,
    dw_merge: jax.Array,
    w_merge: jax.Array,
):
    return _impl(x, w_qkv, w_att_out, w_mlp_in, dw_csgu, w_mlp_out, dw_merge, w_merge)
```

```python
import functools
import math

import jax
import jax.numpy as jnp
import jax.experimental.pallas as pl
import jax.experimental.pallas.tpu as pltpu

_NT = (((1,), (1,)), ((), ()))
_F32 = jnp.float32
_BF16 = jnp.bfloat16


def _make_kernel(B, T, D, K, M, NC, RB, PR, DBG, AU, SV):
    TP = -(-T // 128) * 128
    CK = TP // NC
    PAD = K // 2
    H = 16
    R = T + 2 * H
    M2 = 2 * M
    NS = D // 128
    NPB = T // M2
    NPAIR = B * NPB
    NP = M // PR
    QS = -(-M // 64) * 64
    KP = 32
    eps = 1e-5
    TAPS = [k for b in range(8) for k in range(b, K, 8)]
    qscale = (D ** -0.5) * math.log2(math.e)
    GC1 = math.sqrt(2.0 / math.pi)
    GC2 = GC1 * 0.044715
    NTAIL = NP + 1

    def ln(v, eps=eps):
        mu = jnp.mean(v, axis=-1, keepdims=True)
        c = v - mu
        var = jnp.mean(c * c, axis=-1, keepdims=True)
        return c * jnp.exp2(jnp.log(var + eps) * (-0.5 / math.log(2.0)))

    def kernel(x_hbm, wqkv_hbm, wo_hbm, wmi_hbm, dwc_hbm, wmo_hbm, dwm_hbm, wmg_hbm, out_hbm,
               x_v, o_v, wqkv_v, wo_v, wmo_v, wmg_v, wall, wg, wbc, wbm, k_s, q_s, v_s, u_s, g_s, mg_s, ml_s,
               y_s, dwc_v, dwm_v, zero_s, xsem, osem, wsem, tsem):
        zero_s[0] = 0

        def x_copy(t):
            return pltpu.make_async_copy(x_hbm.at[t], x_v.at[t], xsem.at[t])

        def o_copy(p):
            return pltpu.make_async_copy(o_v.at[p], out_hbm.at[p], osem.at[p])

        def t_copy(i):
            lo, n = (0, M - PR) if i == 0 else (M - PR + (i - 1) * PR, PR)
            return pltpu.make_async_copy(o_v.at[NPAIR - 1, pl.ds(lo, n), :],
                                         out_hbm.at[NPAIR - 1, pl.ds(lo, n), :], tsem.at[i])

        w_copies = [
            pltpu.make_async_copy(wqkv_hbm.at[:, pl.ds(0, 2 * D)], wqkv_v.at[:, pl.ds(0, 2 * D)], wsem.at[0]),
            pltpu.make_async_copy(wmi_hbm.at[:, pl.ds(D, D)], wall.at[:, pl.ds(D, D)], wsem.at[1]),
            pltpu.make_async_copy(wmi_hbm.at[:, pl.ds(0, D)], wall.at[:, pl.ds(2 * D, D)], wsem.at[2]),
            pltpu.make_async_copy(wo_hbm, wo_v, wsem.at[3]),
            pltpu.make_async_copy(dwc_hbm, dwc_v, wsem.at[4]),
            pltpu.make_async_copy(dwm_hbm, dwm_v, wsem.at[5]),
            pltpu.make_async_copy(wmo_hbm, wmo_v, wsem.at[6]),
            pltpu.make_async_copy(wmg_hbm, wmg_v, wsem.at[7]),
            pltpu.make_async_copy(wqkv_hbm.at[:, pl.ds(2 * D, D)], wqkv_v.at[:, pl.ds(2 * D, D)], wsem.at[8]),
        ]
        x_copy(0).start()
        if SV != 1:
            for c in w_copies[:3]:
                c.start()

        zf = jnp.zeros((H, 128), _F32)
        for b in range(B):
            for s in range(NS):
                for m_s in (g_s, mg_s, ml_s):
                    m_s[s, b * R:b * R + H, :] = zf
                    m_s[s, b * R + H + T:(b + 1) * R, :] = zf
                if TP > T:
                    k_s[b, s, T:TP, :] = jnp.zeros((TP - T, 128), _BF16)
            if TP > T:
                v_s[b, T:TP, :] = jnp.zeros((TP - T, 128), _BF16)
        zi = jnp.zeros((PR + 2 * H, 128), _F32)
        for s in range(NS):
            mg_s[s, M2 - PR:M2 + 2 * H, :] = zi
            ml_s[s, M2 - PR:M2 + 2 * H, :] = zi

        def fresh(p):
            return p + zero_s[0]

        cb_cache = {}

        def cbase(p):
            if id(p) not in cb_cache:
                b = p // NPB
                cb_cache[id(p)] = (p, pl.multiple_of(b * R + (p - b * NPB) * M2, 32))
            return cb_cache[id(p)][1]

        def batch_of(p):
            b = 0
            for j in range(1, B):
                b = b + (p >= j * NPB).astype(jnp.int32)
            return b

        def krow_of(t):
            b = batch_of(t)
            return b, pl.multiple_of((t - b * NPB) * M2, 16)

        def a1(t):
            b, krow = krow_of(t)
            xa = ln(x_v[t].astype(_F32))
            for s in range(NS):
                k_s[b, s, pl.ds(krow, M2), :] = xa[:, s * 128:(s + 1) * 128].astype(_BF16)
            lane = jax.lax.broadcasted_iota(jnp.int32, (M2, 128), 1)
            v_s[b, pl.ds(krow, M2), :] = jnp.where(lane == 127, 1.0, xa[:, D - 128:]).astype(_BF16)

        def a2(t):
            b, krow = krow_of(t)
            crow = cbase(t)
            xa = jnp.concatenate([k_s[b, s, pl.ds(krow, M2), :] for s in range(NS)], axis=1)
            y = jnp.dot(xa, wall[...], preferred_element_type=_F32)
            gelu2 = lambda hx: hx * (1.0 + jnp.tanh(hx * (GC1 + GC2 * (hx * hx))))
            u_s[t] = gelu2(y[:, 2 * D:3 * D])
            g = ln(gelu2(y[:, D:2 * D]), 4.0 * eps)
            q = y[:, 0:D]
            for s in range(NS):
                g_s[s, pl.ds(crow + H, M2), :] = g[:, s * 128:(s + 1) * 128]
                for j in range(2):
                    q_s[t, j, s, 0:M, :] = q[j * M:(j + 1) * M, s * 128:(s + 1) * 128].astype(_BF16)

        def late_prep():
            wvo = jnp.dot(wqkv_v[:, 2 * D:3 * D], wo_v[...], preferred_element_type=_F32)
            wg[...] = (wvo - wvo[D - 1:D, :]).astype(_BF16)
            dwc = dwc_v[...].astype(_F32) * 0.5
            dwm = dwm_v[...].astype(_F32)
            for k in range(K):
                for s in range(NS):
                    wbc[s, k] = jnp.broadcast_to(dwc[k:k + 1, s * 128:(s + 1) * 128], (8, 128))
                for s in range(2 * NS):
                    w = dwm[k:k + 1, s * 128:(s + 1) * 128]
                    if k == PAD:
                        w = w + 1.0
                    wbm[s, k] = jnp.broadcast_to(w, (8, 128))

        def phase_a(i, carry):
            for u in range(AU):
                x_copy(i * AU + u + 1).wait()
            if SV >= 3:
                @pl.when(i + 3 < NPAIR)
                def _():
                    x_copy(i + 3).start()

                @pl.when(i == 1)
                def _():
                    for c in w_copies[3:]:
                        c.start()
            for u in range(AU):
                t = i * AU + u
                a2(t)
                a1(jax.lax.rem(t + 1, NPAIR))
            return carry

        x_copy(0).wait()
        if SV == 1:
            for c in w_copies[:3]:
                c.start()
        x_copy(1).start()
        if SV == 2:
            x_copy(2).start()
        a1(fresh(0))
        w_copies[0].wait()
        a = jax.lax.dot_general(wqkv_v[:, 0:D], wqkv_v[:, D:2 * D], _NT, preferred_element_type=_F32) * qscale
        wall[:, 0:D] = a.astype(_BF16)
        w_copies[1].wait()
        w_copies[2].wait()
        if SV < 3:
            for t in range(3 if SV == 2 else 2, NPAIR):
                x_copy(t).start()
            for c in w_copies[3:]:
                c.start()
        else:
            x_copy(2).start()
        NLOOP = (NPAIR - 1) // AU
        jax.lax.fori_loop(0, NLOOP, phase_a, 0)
        if DBG & 2:
            def phase_a2(i, carry):
                for u in range(AU):
                    t = i * AU + u
                    a2(t)
                    a1(jax.lax.rem(t + 1, NPAIR))
                return carry
            jax.lax.fori_loop(0, NLOOP, phase_a2, 0)
        for t in range(NLOOP * AU + 1, NPAIR):
            x_copy(t).wait()
        for c in w_copies[3:]:
            c.wait()
        for t in range(NLOOP * AU, NPAIR):
            a2(fresh(t))
            if t + 1 < NPAIR:
                a1(jax.lax.rem(fresh(t + 1), NPAIR))
        late_prep()

        def conv(src, wb, s, base, off, nrows, ws=0):
            outs = []
            for r in range(nrows // RB):
                acc = None
                for k in TAPS:
                    xk = src[s, pl.ds(base + (off + H + r * RB + k - PAD), RB), :].reshape(RB // 8, 8, 128)
                    term = xk * wb[ws + s, k][None]
                    acc = term if acc is None else acc + term
                outs.append(acc.reshape(RB, 128))
            return jnp.concatenate(outs, axis=0) if len(outs) > 1 else outs[0]

        def att(p, j, hooks):
            crow = cbase(p)
            b = batch_of(p)
            pq = jax.lax.rem(p, NPAIR)
            q = jnp.concatenate([q_s[pq, j, s, 0:M, :] for s in range(NS)], axis=1)

            def qk(c):
                kk = jnp.concatenate([k_s[b, s, c * CK:(c + 1) * CK, :] for s in range(NS)], axis=1)
                s = jax.lax.dot_general(q, kk, _NT, preferred_element_type=_F32)
                if c == NC - 1 and TP > T:
                    lane = jax.lax.broadcasted_iota(jnp.int32, (M, 128), 1)
                    s_last = jnp.where(lane < T - (TP - 128), s[:, CK - 128:], -jnp.inf)
                    s = jnp.concatenate([s[:, :CK - 128], s_last], axis=1)
                return s

            s_next = qk(0)
            for c in range(NC):
                s = s_next
                if c + 1 < NC:
                    s_next = qk(c + 1)
                m_c = jnp.max(s, axis=1, keepdims=True)
                if c == 0:
                    m_new = m_c
                else:
                    m_new = jnp.maximum(m_run, m_c)
                    alpha = jnp.exp2(m_run - m_new)
                pr = jnp.exp2(s - m_new)
                vv = jnp.concatenate([k_s[b, s, c * CK:(c + 1) * CK, :] for s in range(NS - 1)]
                                     + [v_s[b, c * CK:(c + 1) * CK, :]], axis=1)
                pv = jnp.dot(pr.astype(_BF16), vv, preferred_element_type=_F32)
                acc = pv if c == 0 else acc * alpha + pv
                m_run = m_new
                for hk in hooks.get(c, []):
                    hk()
            glob = jnp.dot(acc.astype(_BF16), wg[...], preferred_element_type=_F32) * (1.0 / acc[:, D - 1:D])
            for s in range(NS):
                mg_s[s, pl.ds(crow + (H + j * M), M), :] = glob[:, s * 128:(s + 1) * 128]

        def loc_piece(p, o):
            def h():
                crow = cbase(p)
                gc = jnp.concatenate([conv(g_s, wbc, s, crow, o, PR) for s in range(NS)], axis=1)
                z = (u_s[p, o:o + PR, :] * gc).astype(_BF16)
                y = jnp.dot(z, wmo_v[...], preferred_element_type=_F32)
                for s in range(NS):
                    ml_s[s, pl.ds(crow + (H + o), PR), :] = y[:, s * 128:(s + 1) * 128]
            return h

        def m1_val(p, o):
            mloc = jnp.concatenate([conv(ml_s, wbm, s, cbase(p), o, PR, NS) for s in range(NS)], axis=1).astype(_BF16)
            return x_v[p, o:o + PR, :].astype(_F32) + jnp.dot(mloc, wmg_v[D:2 * D, :], preferred_element_type=_F32)

        def m2_fin(p, o, y1):
            mglob = jnp.concatenate([conv(mg_s, wbm, s, cbase(p), o, PR) for s in range(NS)], axis=1).astype(_BF16)
            y = y1 + jnp.dot(mglob, wmg_v[0:D, :], preferred_element_type=_F32)
            o_v[p, o:o + PR, :] = y.astype(_BF16)

        def merge_pieces(p, o):
            st = []
            return [lambda: st.append(m1_val(p, o)), lambda: m2_fin(p, o, st[0])]

        def m1_stash(p, i):
            def h():
                y_s[i] = m1_val(p, M - PR + i * PR)
            return h

        def body(p, j, merges, locs, stash=False):
            for (pp, o) in merges + locs:
                cbase(pp)
            cbase(p)
            pieces = []
            for (pp, o) in merges:
                pieces += merge_pieces(pp, o)
            pieces += [loc_piece(pp, o) for (pp, o) in locs]
            if stash:
                pieces += [m1_stash(p, i) for i in range(NTAIL)]
            hooks = {}
            n = len(pieces)
            for i, pc in enumerate(pieces):
                c = NC - n + i if n <= NC else (i * NC) // n
                if n < NC - 1:
                    c = 1 + (i * (NC - 1)) // n
                hooks.setdefault(c, []).append(pc)
            att(p, j, hooks)

        def tile_pieces(p, j):
            return [(p, j * M + r * PR) for r in range(NP)]

        def odd_merges(p):
            pm = jnp.maximum(p - 1, 0)
            return [(pm, M2 - PR)] + [(p, r * PR) for r in range(NP - 1)]

        def pair(p, carry):
            @pl.when(p == 0)
            def _():
                p2 = fresh(p)
                body(p2, 0, [], tile_pieces(p2, 0) + tile_pieces(p2, 1))

            @pl.when(p > 0)
            def _():
                p2 = fresh(p)
                pm = p2 - 1
                body(p2, 0, [(pm, M - PR + r * PR) for r in range(NP)], tile_pieces(p2, 1))

            @pl.when(p < NPAIR - 1)
            def _():
                p2 = fresh(p)
                body(p2, 1, odd_merges(p2), tile_pieces(p2 + 1, 0))

            @pl.when(p == NPAIR - 1)
            def _():
                p2 = fresh(p)
                body(p2, 1, odd_merges(p2), [], stash=True)

            @pl.when(p > 0)
            def _():
                o_copy(p - 1).start()
            return carry

        if DBG & 1:
            def fake(p, c):
                z = (u_s[p, 0:16, 0:128] + g_s[0, pl.ds(p * 16, 16), :] + q_s[p, 0, 0, 0:16, :].astype(_F32)
                     + k_s[0, 0, pl.ds(p * 16, 16), :].astype(_F32) + v_s[0, pl.ds(p * 16, 16), :].astype(_F32)
                     + wg[0:16, 0:128].astype(_F32) + wbc[0, p][0:1] + wbm[0, p][0:1])
                o_v[p, 0:16, 0:128] = z.astype(_BF16)
                return c
            jax.lax.fori_loop(0, NPAIR, fake, 0)
            t_copy(1).start()
            t_copy(1).wait()
            return
        jax.lax.fori_loop(0, NPAIR, pair, 0)
        t_copy(0).start()
        pl_ = fresh(NPAIR - 1)
        for i in range(NTAIL):
            m2_fin(pl_, M - PR + i * PR, y_s[i])
            t_copy(i + 1).start()
        for n in range(NPAIR - 1):
            o_copy(n).wait()
        for i in range(NTAIL + 1):
            t_copy(i).wait()

    scratch = [
        pltpu.VMEM((NPAIR, M2, D), _BF16),
        pltpu.VMEM((NPAIR, M2, D), _BF16),
        pltpu.VMEM((D, 3 * D), _BF16),
        pltpu.VMEM((D, D), _BF16),
        pltpu.VMEM((D, D), _BF16),
        pltpu.VMEM((2 * D, D), _BF16),
        pltpu.VMEM((D, 3 * D), _BF16),
        pltpu.VMEM((D, D), _BF16),
        pltpu.VMEM((NS, KP, 8, 128), _F32),
        pltpu.VMEM((2 * NS, KP, 8, 128), _F32),
        pltpu.VMEM((B, NS, TP, 128), _BF16),
        pltpu.VMEM((NPAIR, 2, NS, QS, 128), _BF16),
        pltpu.VMEM((B, TP, 128), _BF16),
        pltpu.VMEM((NPAIR, M2, D), _F32),
        pltpu.VMEM((NS, B * R, 128), _F32),
        pltpu.VMEM((NS, B * R, 128), _F32),
        pltpu.VMEM((NS, B * R, 128), _F32),
        pltpu.VMEM((NTAIL, PR, D), _F32),
        pltpu.VMEM((K, D), _BF16),
        pltpu.VMEM((K, 2 * D), _BF16),
        pltpu.SMEM((1,), jnp.int32),
        pltpu.SemaphoreType.DMA((NPAIR,)),
        pltpu.SemaphoreType.DMA((NPAIR,)),
        pltpu.SemaphoreType.DMA((9,)),
        pltpu.SemaphoreType.DMA((NTAIL + 1,)),
    ]
    return kernel, scratch, NPAIR, M2


def build(M=400, NC=16, RB=80, PR=80, DBG=0, AU=1, SV=0):
    @jax.jit
    def fn(x, w_qkv, w_att_out, w_mlp_in, dw_csgu, w_mlp_out, dw_merge, w_merge):
        B, T, D = x.shape
        K = dw_csgu.shape[0]
        kernel, scratch, NPAIR, M2 = _make_kernel(B, T, D, K, M, NC, RB, PR, DBG, AU, SV)
        out = pl.pallas_call(
            kernel,
            out_shape=jax.ShapeDtypeStruct((NPAIR, M2, D), x.dtype),
            in_specs=[pl.BlockSpec(memory_space=pl.ANY)] * 8,
            out_specs=pl.BlockSpec(memory_space=pl.ANY),
            scratch_shapes=scratch,
            compiler_params=pltpu.CompilerParams(vmem_limit_bytes=110 * 1024 * 1024),
        )(x.reshape(NPAIR, M2, D), w_qkv, w_att_out, w_mlp_in, dw_csgu, w_mlp_out, dw_merge, w_merge)
        return out.reshape(B, T, D)
    return fn


_impl = build(**OPQ)


@jax.jit
def pallas_standalone__conformer_family_e_branchformer__speech_kernel(
    x: jax.Array,
    w_qkv: jax.Array,
    w_att_out: jax.Array,
    w_mlp_in: jax.Array,
    dw_csgu: jax.Array,
    w_mlp_out: jax.Array,
    dw_merge: jax.Array,
    w_merge: jax.Array,
):
    return _impl(x, w_qkv, w_att_out, w_mlp_in, dw_csgu, w_mlp_out, dw_merge, w_merge)
```

```python
import math

import jax
import jax.numpy as jnp
import jax.experimental.pallas as pl
import jax.experimental.pallas.tpu as pltpu

_NT = (((1,), (1,)), ((), ()))
_F32 = jnp.float32
_BF16 = jnp.bfloat16


def _up(a, m):
    return -(-a // m) * m


def _make_kernel(B, T, D, K, M, NC, PR, ML, DBG):
    TP = _up(T, 128)
    CK = TP // NC
    PAD = K // 2
    H = 16
    SL = _up(M + 2 * H, 32)
    XS = _up(M, 32)
    QS = _up(M, 64)
    NS = D // 128
    NTB = T // M
    NT = B * NTB
    NA = NT // 2
    NP = M // PR
    KP = _up(K, 32)
    NST = NP + 1
    NTAIL = ML // PR + 1
    TLO = M - NTAIL * PR
    eps = 1e-5
    taps = [k for b in range(8) for k in range(b, K, 8)]
    qscale = (D ** -0.5) * math.log2(math.e)
    gc1 = math.sqrt(2.0 / math.pi)
    gc2 = gc1 * 0.044715
    assert T % (2 * M) == 0 and M % PR == 0 and PR % 16 == 0 and ML % PR == 0 and PAD <= H
    assert TP - T < 128 and TP % NC == 0 and CK % 128 == 0 and NS >= 2 and NT >= 4

    def gelu2(h):
        return h * (1.0 + jnp.tanh(h * (gc1 + gc2 * (h * h))))

    def ln(v, e):
        mu = jnp.mean(v, axis=-1, keepdims=True)
        c = v - mu
        var = jnp.mean(c * c, axis=-1, keepdims=True)
        return c * jnp.exp2(jnp.log(var + e) * (-0.5 / math.log(2.0)))

    def kernel(x_hbm, wqkv_hbm, wo_hbm, wmi_hbm, dwc_hbm, wmo_hbm, dwm_hbm, wmg_hbm, out_hbm,
               x_v, o_v, wqkv_v, wo_v, wmo_v, wmg_v, wall, wg, wbc, wbm, k_s, q_s, v_s, u_s,
               g_s, mg_s, ml_s, y_s, dwc_v, dwm_v, zero_s, xsem, wsem, osem):
        zero_s[0] = 0

        def x_copy(t):
            return pltpu.make_async_copy(x_hbm.at[pl.ds(2 * t, 2)],
                                         x_v.at[pl.ds(2 * t, 2), pl.ds(0, M), :], xsem.at[t])

        def o_copy(n, lo=0, cnt=M):
            return pltpu.make_async_copy(o_v.at[n, pl.ds(lo, cnt), :],
                                         out_hbm.at[n, pl.ds(lo, cnt), :], osem.at[0])

        wqk_copy = pltpu.make_async_copy(wqkv_hbm.at[:, pl.ds(0, 2 * D)],
                                         wqkv_v.at[:, pl.ds(0, 2 * D)], wsem.at[0])
        wmi_copies = [
            pltpu.make_async_copy(wmi_hbm.at[:, pl.ds(D, D)], wall.at[:, pl.ds(D, D)], wsem.at[1]),
            pltpu.make_async_copy(wmi_hbm.at[:, pl.ds(0, D)], wall.at[:, pl.ds(2 * D, D)], wsem.at[1]),
        ]
        late_copies = [
            pltpu.make_async_copy(wqkv_hbm.at[:, pl.ds(2 * D, D)], wqkv_v.at[:, pl.ds(2 * D, D)], wsem.at[2]),
            pltpu.make_async_copy(wo_hbm, wo_v, wsem.at[2]),
            pltpu.make_async_copy(dwc_hbm, dwc_v, wsem.at[2]),
            pltpu.make_async_copy(dwm_hbm, dwm_v, wsem.at[2]),
            pltpu.make_async_copy(wmo_hbm, wmo_v, wsem.at[2]),
            pltpu.make_async_copy(wmg_hbm, wmg_v, wsem.at[2]),
        ]
        x_copy(0).start()
        wqk_copy.start()
        for c in wmi_copies:
            c.start()
        for t in range(1, NA):
            x_copy(t).start()
        for c in late_copies:
            c.start()

        zh = jnp.zeros((H, 128), _F32)
        for b in range(B):
            first, last = (b * (NTB + 1) + 1) * SL, (b + 1) * (NTB + 1) * SL - SL
            for s in range(NS):
                for arr in (g_s, mg_s, ml_s):
                    arr[s, first:first + H, :] = zh
                    arr[s, last + H + M:last + 2 * H + M, :] = zh
                if TP > T:
                    k_s[b, s, T:TP, :] = jnp.zeros((TP - T, 128), _BF16)
            if TP > T:
                v_s[b, T:TP, :] = jnp.zeros((TP - T, 128), _BF16)
        for s in range(NS):
            mg_s[s, SL + H + M:SL + 2 * H + M, :] = zh

        def fresh(n):
            return jax.lax.rem(n + zero_s[0], 2 * NT)

        def batch_of(n, per):
            b = 0
            for j in range(1, B):
                b = b + (n >= j * per).astype(jnp.int32)
            return b

        slots = {}

        def slot(n):
            if id(n) not in slots:
                slots[id(n)] = (n, pl.multiple_of((n + batch_of(n, NTB)) * SL, 32))
            return slots[id(n)][1]

        def put(arr, n, lo, val, j=0):
            cnt = val.shape[0]
            base = slot(n)
            s0 = (j + 1) * SL
            for s in range(NS):
                v = val[:, s * 128:(s + 1) * 128]
                arr[s, pl.ds(base + (s0 + H + lo), cnt), :] = v
                if lo == 0:
                    arr[s, pl.ds(base + (s0 - SL + H + M), H), :] = v[0:H]
                if lo + cnt == M:
                    arr[s, pl.ds(base + (s0 + SL), H), :] = v[cnt - H:cnt]

        def krow_of(t):
            b = batch_of(t, NA // B)
            return b, pl.multiple_of((t - b * (NA // B)) * (2 * M), 16)

        def a1(t):
            b, krow = krow_of(t)
            x = jnp.concatenate([x_v[2 * t + j, 0:M, :] for j in range(2)], axis=0)
            xa = ln(x.astype(_F32), eps)
            for s in range(NS):
                k_s[b, s, pl.ds(krow, 2 * M), :] = xa[:, s * 128:(s + 1) * 128].astype(_BF16)
            lane = jax.lax.broadcasted_iota(jnp.int32, (2 * M, 128), 1)
            v_s[b, pl.ds(krow, 2 * M), :] = jnp.where(lane == 127, 1.0, xa[:, D - 128:]).astype(_BF16)

        def a2(t):
            b, krow = krow_of(t)
            xa = jnp.concatenate([k_s[b, s, pl.ds(krow, 2 * M), :] for s in range(NS)], axis=1)
            y = jnp.dot(xa, wall[...], preferred_element_type=_F32)
            g = ln(gelu2(y[:, D:2 * D]), 4.0 * eps)
            n0 = 2 * t
            for j in range(2):
                rows = slice(j * M, (j + 1) * M)
                u_s[2 * t + j] = y[rows, 2 * D:3 * D]
                put(g_s, n0, 0, g[rows], j)
                for s in range(NS):
                    q_s[2 * t + j, s, 0:M, :] = y[rows, s * 128:(s + 1) * 128].astype(_BF16)

        def late_prep():
            wvo = jnp.dot(wqkv_v[:, 2 * D:3 * D], wo_v[...], preferred_element_type=_F32)
            wg[...] = (wvo - wvo[D - 1:D, :]).astype(_BF16)
            dwc = dwc_v[...].astype(_F32) * 0.5
            dwm = dwm_v[...].astype(_F32)
            for k in range(K):
                for s in range(NS):
                    wbc[s, k] = jnp.broadcast_to(dwc[k:k + 1, s * 128:(s + 1) * 128], (8, 128))
                for s in range(2 * NS):
                    w = dwm[k:k + 1, s * 128:(s + 1) * 128]
                    if k == PAD:
                        w = w + 1.0
                    wbm[s, k] = jnp.broadcast_to(w, (8, 128))

        def phase_a(t, carry):
            x_copy(t + 1).wait()
            a2(t)
            a1(fresh(t + 1))
            return carry

        x_copy(0).wait()
        a1(fresh(0))
        wqk_copy.wait()
        a = jax.lax.dot_general(wqkv_v[:, 0:D], wqkv_v[:, D:2 * D], _NT, preferred_element_type=_F32)
        wall[:, 0:D] = (a * qscale).astype(_BF16)
        for c in wmi_copies:
            c.wait()
        jax.lax.fori_loop(0, NA - 1, phase_a, 0)
        for c in late_copies:
            c.wait()
        a2(fresh(NA - 1))
        late_prep()

        def conv(src, wb, ws, n, o):
            base = slot(n)
            outs = []
            for s in range(NS):
                acc = None
                for k in taps:
                    xk = src[s, pl.ds(base + (SL + o + H + k - PAD), PR), :].reshape(PR // 8, 8, 128)
                    term = xk * wb[ws + s, k][None]
                    acc = term if acc is None else acc + term
                outs.append(acc.reshape(PR, 128))
            return jnp.concatenate(outs, axis=1)

        def loc_piece(n, o):
            def run():
                z = (gelu2(u_s[n, o:o + PR, :]) * conv(g_s, wbc, 0, n, o)).astype(_BF16)
                put(ml_s, n, o, jnp.dot(z, wmo_v[...], preferred_element_type=_F32))
            return run

        def merge_loc(n, o):
            m = conv(ml_s, wbm, NS, n, o).astype(_BF16)
            return (x_v[n, o:o + PR, :].astype(_F32)
                    + jnp.dot(m, wmg_v[D:2 * D, :], preferred_element_type=_F32))

        def merge_glob(n, o, y1):
            m = conv(mg_s, wbm, 0, n, o).astype(_BF16)
            y = y1 + jnp.dot(m, wmg_v[0:D, :], preferred_element_type=_F32)
            o_v[n, o:o + PR, :] = y.astype(_BF16)

        def locs(n):
            slot(n)
            return [loc_piece(n, r * PR) for r in range(NP)]

        def merges(n):
            n2 = jnp.maximum(n - 2, 0)
            n1 = n - 1
            slot(n2)
            slot(n1)
            out = []
            for (nn, o) in [(n2, M - PR)] + [(n1, r * PR) for r in range(NP - 1)]:
                def two(nn=nn, o=o):
                    st = []
                    return [lambda: st.append(merge_loc(nn, o)), lambda: merge_glob(nn, o, st[0])]
                out += two()
            return out

        def end_loc(n, i):
            nn, o = (n - 1, M - PR) if i == 0 else (n, (i - 1) * PR)
            slot(nn)
            return nn, o

        def stash(n, i):
            nn, o = end_loc(n, i)

            def run():
                y_s[i] = merge_loc(nn, o)
            return run

        def finish(n, i):
            nn, o = end_loc(n, i)
            return lambda: merge_glob(nn, o, y_s[i])

        def attend(n, b, off, mr, pieces):
            hooks = {}
            cnt = len(pieces)
            for i, pc in enumerate(pieces):
                if cnt < NC - 1:
                    c = 1 + (i * (NC - 1)) // cnt
                elif cnt <= NC:
                    c = NC - cnt + i
                else:
                    c = (i * NC) // cnt
                hooks.setdefault(c, []).append(pc)

            q = jnp.concatenate([q_s[n, s, off:off + mr, :] for s in range(NS)], axis=1)

            def qk(c):
                kk = jnp.concatenate([k_s[b, s, c * CK:(c + 1) * CK, :] for s in range(NS)], axis=1)
                s = jax.lax.dot_general(q, kk, _NT, preferred_element_type=_F32)
                if c == NC - 1 and TP > T:
                    lane = jax.lax.broadcasted_iota(jnp.int32, (mr, 128), 1)
                    s_last = jnp.where(lane < T - (TP - 128), s[:, CK - 128:], -jnp.inf)
                    s = jnp.concatenate([s[:, :CK - 128], s_last], axis=1)
                return s

            s_next = qk(0)
            for c in range(NC):
                s = s_next
                if c + 1 < NC:
                    s_next = qk(c + 1)
                m_c = jnp.max(s, axis=1, keepdims=True)
                if c == 0:
                    m_new = m_c
                else:
                    m_new = jnp.maximum(m_run, m_c)
                    alpha = jnp.exp2(m_run - m_new)
                pr = jnp.exp2(s - m_new)
                vv = jnp.concatenate([k_s[b, s_, c * CK:(c + 1) * CK, :] for s_ in range(NS - 1)]
                                     + [v_s[b, c * CK:(c + 1) * CK, :]], axis=1)
                pv = jnp.dot(pr.astype(_BF16), vv, preferred_element_type=_F32)
                acc = pv if c == 0 else acc * alpha + pv
                m_run = m_new
                for hk in hooks.get(c, []):
                    hk()
            glob = jnp.dot(acc.astype(_BF16), wg[...], preferred_element_type=_F32)
            put(mg_s, n, off, glob * (1.0 / acc[:, D - 1:D]))

        def block(always):
            return pl.when(zero_s[0] == 0)(always)

        @block
        def _():
            n = fresh(0)
            attend(n, 0, 0, M, locs(n) + locs(n + 1))

        def tile(i, carry):
            n = fresh(i)
            attend(n, batch_of(i, NTB), 0, M, merges(n) + locs(n + 1))

            @pl.when(i >= 2)
            def _():
                o_copy(i - 2).start()
            return carry

        jax.lax.fori_loop(1, NT - 1, tile, 0)

        n = fresh(NT - 1)
        attend(n, B - 1, 0, M - ML, merges(n) + [stash(n, i) for i in range(NST)])
        o_copy(NT - 3).start()

        @block
        def _():
            n = fresh(NT - 1)
            attend(n, B - 1, M - ML, ML, [finish(n, i) for i in range(NST - NTAIL)])
            o_copy(NT - 2).start()
            o_copy(NT - 1, 0, TLO).start()

        n = fresh(NT - 1)
        for i in range(NTAIL):
            finish(n, NST - NTAIL + i)()
            o_copy(NT - 1, TLO + i * PR, PR).start()

        for i in range(NT - 1):
            o_copy(i).wait()
        o_copy(NT - 1, 0, TLO).wait()
        for i in range(NTAIL):
            o_copy(NT - 1, TLO + i * PR, PR).wait()

    scratch = [
        pltpu.VMEM((NT, XS, D), _BF16),
        pltpu.VMEM((NT, XS, D), _BF16),
        pltpu.VMEM((D, 3 * D), _BF16),
        pltpu.VMEM((D, D), _BF16),
        pltpu.VMEM((D, D), _BF16),
        pltpu.VMEM((2 * D, D), _BF16),
        pltpu.VMEM((D, 3 * D), _BF16),
        pltpu.VMEM((D, D), _BF16),
        pltpu.VMEM((NS, KP, 8, 128), _F32),
        pltpu.VMEM((2 * NS, KP, 8, 128), _F32),
        pltpu.VMEM((B, NS, TP, 128), _BF16),
        pltpu.VMEM((NT, NS, QS, 128), _BF16),
        pltpu.VMEM((B, TP, 128), _BF16),
        pltpu.VMEM((NT, M, D), _F32),
        pltpu.VMEM((NS, (NT + B + 1) * SL, 128), _F32),
        pltpu.VMEM((NS, (NT + B + 1) * SL, 128), _F32),
        pltpu.VMEM((NS, (NT + B + 1) * SL, 128), _F32),
        pltpu.VMEM((NST, PR, D), _F32),
        pltpu.VMEM((K, D), _BF16),
        pltpu.VMEM((K, 2 * D), _BF16),
        pltpu.SMEM((1,), jnp.int32),
        pltpu.SemaphoreType.DMA((NA,)),
        pltpu.SemaphoreType.DMA((3,)),
        pltpu.SemaphoreType.DMA((1,)),
    ]
    return kernel, scratch, NT


def build(M=400, NC=16, PR=80, ML=160, DBG=0):
    @jax.jit
    def fn(x, w_qkv, w_att_out, w_mlp_in, dw_csgu, w_mlp_out, dw_merge, w_merge):
        B, T, D = x.shape
        K = dw_csgu.shape[0]
        kernel, scratch, NT = _make_kernel(B, T, D, K, M, NC, PR, ML, DBG)
        out = pl.pallas_call(
            kernel,
            out_shape=jax.ShapeDtypeStruct((NT, M, D), x.dtype),
            in_specs=[pl.BlockSpec(memory_space=pl.ANY)] * 8,
            out_specs=pl.BlockSpec(memory_space=pl.ANY),
            scratch_shapes=scratch,
            compiler_params=pltpu.CompilerParams(vmem_limit_bytes=110 * 1024 * 1024),
        )(x.reshape(NT, M, D), w_qkv, w_att_out, w_mlp_in, dw_csgu, w_mlp_out, dw_merge, w_merge)
        return out.reshape(B, T, D)
    return fn


_impl = build(**OPQ)


@jax.jit
def pallas_standalone__conformer_family_e_branchformer__speech_kernel(
    x: jax.Array,
    w_qkv: jax.Array,
    w_att_out: jax.Array,
    w_mlp_in: jax.Array,
    dw_csgu: jax.Array,
    w_mlp_out: jax.Array,
    dw_merge: jax.Array,
    w_merge: jax.Array,
):
    return _impl(x, w_qkv, w_att_out, w_mlp_in, dw_csgu, w_mlp_out, dw_merge, w_merge)
```

```python
import math

import jax
import jax.numpy as jnp
import jax.experimental.pallas as pl
import jax.experimental.pallas.tpu as pltpu

_NT = (((1,), (1,)), ((), ()))
_F32 = jnp.float32
_BF16 = jnp.bfloat16

_M = 400
_CK = 512
_PR = 80
_ML = 80


def _up(a, m):
    return -(-a // m) * m


def _make_kernel(B, T, D, K):
    M, PR, ML = _M, _PR, _ML
    TP = _up(T, _CK)
    CK = _CK
    NC = TP // CK
    PAD = K // 2
    H = 16
    SL = _up(M + 2 * H, 32)
    XS = _up(M, 32)
    QS = _up(M, 64)
    NS = D // 128
    NTB = T // M
    NT = B * NTB
    NA = NT // 2
    NP = M // PR
    KP = _up(K, 32)
    NST = NP + 1
    NTAIL = ML // PR + 1
    TLO = M - NTAIL * PR
    eps = 1e-5
    taps = [k for b in range(8) for k in range(b, K, 8)]
    qscale = (D ** -0.5) * math.log2(math.e)
    gc1 = math.sqrt(2.0 / math.pi)
    gc2 = gc1 * 0.044715
    assert T % (2 * M) == 0 and M % PR == 0 and PR % 16 == 0 and ML % PR == 0 and PAD <= H
    assert TP - T < 128 and D % 128 == 0 and NS >= 2 and NT >= 4 and NC >= 2

    def gelu2(h):
        return h * (1.0 + jnp.tanh(h * (gc1 + gc2 * (h * h))))

    def ln(v, e):
        mu = jnp.mean(v, axis=-1, keepdims=True)
        c = v - mu
        var = jnp.mean(c * c, axis=-1, keepdims=True)
        return c * jnp.exp2(jnp.log(var + e) * (-0.5 / math.log(2.0)))

    def kernel(x_hbm, wqkv_hbm, wo_hbm, wmi_hbm, dwc_hbm, wmo_hbm, dwm_hbm, wmg_hbm, out_hbm,
               x_v, o_v, wqkv_v, wo_v, wmo_v, wmg_v, wall, wg, wbc, wbm, k_s, q_s, v_s, u_s,
               g_s, mg_s, ml_s, y_s, kt_s, dwc_v, dwm_v, zero_s, xsem, wsem, osem):
        zero_s[0] = 0

        def x_copy(t):
            return pltpu.make_async_copy(x_hbm.at[pl.ds(2 * t, 2)],
                                         x_v.at[pl.ds(2 * t, 2), pl.ds(0, M), :], xsem.at[t])

        def h_copy(j):
            return pltpu.make_async_copy(x_hbm.at[j], x_v.at[j, pl.ds(0, M), :],
                                         xsem.at[0 if j == 0 else NA])

        def o_copy(n, lo=0, cnt=M):
            return pltpu.make_async_copy(o_v.at[n, pl.ds(lo, cnt), :],
                                         out_hbm.at[n, pl.ds(lo, cnt), :], osem.at[0])

        wqk_copy = pltpu.make_async_copy(wqkv_hbm.at[:, pl.ds(0, 2 * D)],
                                         wqkv_v.at[:, pl.ds(0, 2 * D)], wsem.at[0])
        wmi_copies = [
            pltpu.make_async_copy(wmi_hbm.at[:, pl.ds(D, D)], wall.at[:, pl.ds(D, D)], wsem.at[1]),
            pltpu.make_async_copy(wmi_hbm.at[:, pl.ds(0, D)], wall.at[:, pl.ds(2 * D, D)], wsem.at[1]),
        ]
        late_copies = [
            pltpu.make_async_copy(wqkv_hbm.at[:, pl.ds(2 * D, D)], wqkv_v.at[:, pl.ds(2 * D, D)],
                                  wsem.at[2]),
            pltpu.make_async_copy(wo_hbm, wo_v, wsem.at[2]),
            pltpu.make_async_copy(dwc_hbm, dwc_v, wsem.at[2]),
            pltpu.make_async_copy(dwm_hbm, dwm_v, wsem.at[2]),
            pltpu.make_async_copy(wmo_hbm, wmo_v, wsem.at[2]),
            pltpu.make_async_copy(wmg_hbm, wmg_v, wsem.at[2]),
        ]
        h_copy(0).start()
        wqk_copy.start()
        for c in wmi_copies:
            c.start()
        h_copy(1).start()

        zh = jnp.zeros((H, 128), _F32)
        for b in range(B):
            first, last = (b * (NTB + 1) + 1) * SL, (b + 1) * (NTB + 1) * SL - SL
            for s in range(NS):
                for arr in (g_s, mg_s, ml_s):
                    arr[s, first:first + H, :] = zh
                    arr[s, last + H + M:last + 2 * H + M, :] = zh
                if TP > T:
                    k_s[b, s, T:TP, :] = jnp.zeros((TP - T, 128), _BF16)
            if TP > T:
                v_s[b, T:TP, :] = jnp.zeros((TP - T, 128), _BF16)
        for s in range(NS):
            mg_s[s, SL + H + M:SL + 2 * H + M, :] = zh

        def fresh(n):
            return jax.lax.rem(n + zero_s[0], 2 * NT)

        def batch_of(n, per):
            b = 0
            for j in range(1, B):
                b = b + (n >= j * per).astype(jnp.int32)
            return b

        slots = {}

        def slot(n):
            if id(n) not in slots:
                slots[id(n)] = (n, pl.multiple_of((n + batch_of(n, NTB)) * SL, 32))
            return slots[id(n)][1]

        def put(arr, n, lo, val, j=0):
            cnt = val.shape[0]
            base = slot(n)
            s0 = (j + 1) * SL
            for s in range(NS):
                v = val[:, s * 128:(s + 1) * 128]
                arr[s, pl.ds(base + (s0 + H + lo), cnt), :] = v
                if lo == 0:
                    arr[s, pl.ds(base + (s0 - SL + H + M), H), :] = v[0:H]
                if lo + cnt == M:
                    arr[s, pl.ds(base + (s0 + SL), H), :] = v[cnt - H:cnt]

        def krow_of(t):
            b = batch_of(t, NA // B)
            return b, pl.multiple_of((t - b * (NA // B)) * (2 * M), 16)

        def a1(t, js=(0, 1)):
            b, krow = krow_of(t)
            lo, cnt = js[0] * M, len(js) * M
            x = jnp.concatenate([x_v[2 * t + j, 0:M, :] for j in js], axis=0)
            xa = ln(x.astype(_F32), eps)
            for s in range(NS):
                k_s[b, s, pl.ds(krow + lo, cnt), :] = xa[:, s * 128:(s + 1) * 128].astype(_BF16)
            lane = jax.lax.broadcasted_iota(jnp.int32, (cnt, 128), 1)
            v_s[b, pl.ds(krow + lo, cnt), :] = jnp.where(lane == 127, 1.0, xa[:, D - 128:]).astype(_BF16)

        def a2(t, js=(0, 1)):
            b, krow = krow_of(t)
            lo, cnt = js[0] * M, len(js) * M
            xa = jnp.concatenate([k_s[b, s, pl.ds(krow + lo, cnt), :] for s in range(NS)], axis=1)
            y = jnp.dot(xa, wall[...], preferred_element_type=_F32)
            g = ln(gelu2(y[:, D:2 * D]), 4.0 * eps)
            n0 = 2 * t
            for j in js:
                rows = slice(j * M - lo, (j + 1) * M - lo)
                u_s[2 * t + j] = y[rows, 2 * D:3 * D]
                put(g_s, n0, 0, g[rows], j)
                for s in range(NS):
                    q_s[2 * t + j, s, 0:M, :] = y[rows, s * 128:(s + 1) * 128].astype(_BF16)

        def late_prep():
            for b in range(B):
                k0 = jnp.concatenate([k_s[b, s, 0:CK, :] for s in range(NS)], axis=1)
                kt_s[b] = k0.astype(_F32).T.astype(_BF16)
            wvo = jnp.dot(wqkv_v[:, 2 * D:3 * D], wo_v[...], preferred_element_type=_F32)
            wg[...] = (wvo - wvo[D - 1:D, :]).astype(_BF16)
            dwc = dwc_v[...].astype(_F32) * 0.5
            dwm = dwm_v[...].astype(_F32)
            for k in range(K):
                for s in range(NS):
                    wbc[s, k] = jnp.broadcast_to(dwc[k:k + 1, s * 128:(s + 1) * 128], (8, 128))
                for s in range(2 * NS):
                    w = dwm[k:k + 1, s * 128:(s + 1) * 128]
                    if k == PAD:
                        w = w + 1.0
                    wbm[s, k] = jnp.broadcast_to(w, (8, 128))

        def phase_a(t, carry):
            x_copy(t + 1).wait()
            a2(t)
            a1(fresh(t + 1))
            return carry

        h_copy(0).wait()
        x_copy(1).start()
        a1(fresh(0), (0,))
        wqk_copy.wait()
        a = jax.lax.dot_general(wqkv_v[:, 0:D], wqkv_v[:, D:2 * D], _NT, preferred_element_type=_F32)
        wall[:, 0:D] = (a * qscale).astype(_BF16)
        for c in wmi_copies:
            c.wait()
        h_copy(1).wait()
        a2(fresh(0), (0,))
        a1(fresh(0), (1,))
        x_copy(1).wait()
        for t in range(2, NA):
            x_copy(t).start()
        for c in late_copies:
            c.start()
        a2(fresh(0), (1,))
        a1(fresh(1))
        jax.lax.fori_loop(1, NA - 1, phase_a, 0)
        for c in late_copies:
            c.wait()
        a2(fresh(NA - 1))
        late_prep()

        def conv(src, wb, ws, n, o):
            base = slot(n)
            outs = []
            for s in range(NS):
                acc = None
                for k in taps:
                    xk = src[s, pl.ds(base + (SL + o + H + k - PAD), PR), :].reshape(PR // 8, 8, 128)
                    term = xk * wb[ws + s, k][None]
                    acc = term if acc is None else acc + term
                outs.append(acc.reshape(PR, 128))
            return jnp.concatenate(outs, axis=1)

        def loc_piece(n, o):
            def run():
                z = (gelu2(u_s[n, o:o + PR, :]) * conv(g_s, wbc, 0, n, o)).astype(_BF16)
                put(ml_s, n, o, jnp.dot(z, wmo_v[...], preferred_element_type=_F32))
            return run

        def merge_loc(n, o):
            m = conv(ml_s, wbm, NS, n, o).astype(_BF16)
            return (x_v[n, o:o + PR, :].astype(_F32)
                    + jnp.dot(m, wmg_v[D:2 * D, :], preferred_element_type=_F32))

        def merge_glob(n, o, y1):
            m = conv(mg_s, wbm, 0, n, o).astype(_BF16)
            y = y1 + jnp.dot(m, wmg_v[0:D, :], preferred_element_type=_F32)
            o_v[n, o:o + PR, :] = y.astype(_BF16)

        def locs(n):
            slot(n)
            return [loc_piece(n, r * PR) for r in range(NP)]

        def merges(n):
            n2 = jnp.maximum(n - 2, 0)
            n1 = n - 1
            slot(n2)
            slot(n1)
            out = []
            for (nn, o) in [(n2, M - PR)] + [(n1, r * PR) for r in range(NP - 1)]:
                def two(nn=nn, o=o):
                    st = []
                    return [lambda: st.append(merge_loc(nn, o)), lambda: merge_glob(nn, o, st[0])]
                out += two()
            return out

        def end_loc(n, i):
            nn, o = (n - 1, M - PR) if i == 0 else (n, (i - 1) * PR)
            slot(nn)
            return nn, o

        def stash(n, i):
            nn, o = end_loc(n, i)

            def run():
                y_s[i] = merge_loc(nn, o)
            return run

        def finish(n, i):
            nn, o = end_loc(n, i)
            return lambda: merge_glob(nn, o, y_s[i])

        def attend(n, b, off, mr, pieces):
            hooks = {}
            cnt = len(pieces)
            for i, pc in enumerate(pieces):
                if cnt == 2 * NC - 1:
                    h = i + 1
                else:
                    done = lambda h: min(h // 2 + 2, NC) + (h + 1) // 2
                    want = (i + 3) * (2 * NC) / (cnt + 2)
                    h = min((h for h in range(2 * NC) if h != 2 * NC - 2),
                            key=lambda h: abs(done(h) - want))
                hooks.setdefault(h, []).append(pc)

            q = jnp.concatenate([q_s[n, s, off:off + mr, :] for s in range(NS)], axis=1)

            def qk(c):
                if c == 0:
                    return jnp.dot(q, kt_s[b], preferred_element_type=_F32)
                kk = jnp.concatenate([k_s[b, s, c * CK:(c + 1) * CK, :] for s in range(NS)], axis=1)
                s = jax.lax.dot_general(q, kk, _NT, preferred_element_type=_F32)
                if c == NC - 1 and TP > T:
                    lane = jax.lax.broadcasted_iota(jnp.int32, (mr, 128), 1)
                    s_last = jnp.where(lane < T - (TP - 128), s[:, CK - 128:], -jnp.inf)
                    s = jnp.concatenate([s[:, :CK - 128], s_last], axis=1)
                return s

            s_next = qk(0)
            for c in range(NC):
                s = s_next
                if c + 1 < NC:
                    s_next = qk(c + 1)
                for hk in hooks.get(2 * c, []):
                    hk()
                m_c = jnp.max(s, axis=1, keepdims=True)
                if c == 0:
                    m_new = m_c
                else:
                    m_new = jnp.maximum(m_run, m_c)
                    alpha = jnp.exp2(m_run - m_new)
                pr = jnp.exp2(s - m_new)
                vv = jnp.concatenate([k_s[b, s_, c * CK:(c + 1) * CK, :] for s_ in range(NS - 1)]
                                     + [v_s[b, c * CK:(c + 1) * CK, :]], axis=1)
                pv = jnp.dot(pr.astype(_BF16), vv, preferred_element_type=_F32)
                acc = pv if c == 0 else acc * alpha + pv
                m_run = m_new
                for hk in hooks.get(2 * c + 1, []):
                    hk()
            glob = jnp.dot(acc.astype(_BF16), wg[...], preferred_element_type=_F32)
            put(mg_s, n, off, glob * (1.0 / acc[:, D - 1:D]))

        def block(fn):
            return pl.when(zero_s[0] == 0)(fn)

        @block
        def _():
            n = fresh(0)
            attend(n, 0, 0, M, locs(n) + locs(n + 1))

        def tile(i, carry):
            n = fresh(i)
            attend(n, batch_of(i, NTB), 0, M, merges(n) + locs(n + 1))

            @pl.when(i >= 2)
            def _():
                o_copy(i - 2).start()
            return carry

        jax.lax.fori_loop(1, NT - 1, tile, 0)

        n = fresh(NT - 1)
        attend(n, B - 1, 0, M - ML, merges(n) + [stash(n, i) for i in range(NST)])
        o_copy(NT - 3).start()

        @block
        def _():
            n = fresh(NT - 1)
            attend(n, B - 1, M - ML, ML, [finish(n, i) for i in range(NST - NTAIL)])
            o_copy(NT - 2).start()
            o_copy(NT - 1, 0, TLO).start()

        n = fresh(NT - 1)
        for i in range(NTAIL):
            finish(n, NST - NTAIL + i)()
            o_copy(NT - 1, TLO + i * PR, PR).start()

        for i in range(NT - 1):
            o_copy(i).wait()
        o_copy(NT - 1, 0, TLO).wait()
        for i in range(NTAIL):
            o_copy(NT - 1, TLO + i * PR, PR).wait()

    scratch = [
        pltpu.VMEM((NT, XS, D), _BF16),
        pltpu.VMEM((NT, XS, D), _BF16),
        pltpu.VMEM((D, 3 * D), _BF16),
        pltpu.VMEM((D, D), _BF16),
        pltpu.VMEM((D, D), _BF16),
        pltpu.VMEM((2 * D, D), _BF16),
        pltpu.VMEM((D, 3 * D), _BF16),
        pltpu.VMEM((D, D), _BF16),
        pltpu.VMEM((NS, KP, 8, 128), _F32),
        pltpu.VMEM((2 * NS, KP, 8, 128), _F32),
        pltpu.VMEM((B, NS, TP, 128), _BF16),
        pltpu.VMEM((NT, NS, QS, 128), _BF16),
        pltpu.VMEM((B, TP, 128), _BF16),
        pltpu.VMEM((NT, M, D), _F32),
        pltpu.VMEM((NS, (NT + B + 1) * SL, 128), _F32),
        pltpu.VMEM((NS, (NT + B + 1) * SL, 128), _F32),
        pltpu.VMEM((NS, (NT + B + 1) * SL, 128), _F32),
        pltpu.VMEM((NST, PR, D), _F32),
        pltpu.VMEM((B, D, CK), _BF16),
        pltpu.VMEM((K, D), _BF16),
        pltpu.VMEM((K, 2 * D), _BF16),
        pltpu.SMEM((1,), jnp.int32),
        pltpu.SemaphoreType.DMA((NA + 1,)),
        pltpu.SemaphoreType.DMA((3,)),
        pltpu.SemaphoreType.DMA((1,)),
    ]
    return kernel, scratch, NT


@jax.jit
def pallas_standalone__conformer_family_e_branchformer__speech_kernel(
    x: jax.Array,
    w_qkv: jax.Array,
    w_att_out: jax.Array,
    w_mlp_in: jax.Array,
    dw_csgu: jax.Array,
    w_mlp_out: jax.Array,
    dw_merge: jax.Array,
    w_merge: jax.Array,
):
    B, T, D = x.shape
    K = dw_csgu.shape[0]
    kernel, scratch, NT = _make_kernel(B, T, D, K)
    out = pl.pallas_call(
        kernel,
        out_shape=jax.ShapeDtypeStruct((NT, _M, D), x.dtype),
        in_specs=[pl.BlockSpec(memory_space=pl.ANY)] * 8,
        out_specs=pl.BlockSpec(memory_space=pl.ANY),
        scratch_shapes=scratch,
        compiler_params=pltpu.CompilerParams(vmem_limit_bytes=110 * 1024 * 1024),
    )(x.reshape(NT, _M, D), w_qkv, w_att_out, w_mlp_in, dw_csgu, w_mlp_out, dw_merge, w_merge)
    return out.reshape(B, T, D)
```

```python
import math

import jax
import jax.numpy as jnp
import jax.experimental.pallas as pl
import jax.experimental.pallas.tpu as pltpu

_NT = (((1,), (1,)), ((), ()))
_F32 = jnp.float32
_BF16 = jnp.bfloat16

_M = 400
_CK = 512
_PR = 80
_ML = 80


def _up(a, m):
    return -(-a // m) * m


def _make_kernel(B, T, D, K):
    M, PR, ML = _M, _PR, _ML
    TP = _up(T, _CK)
    CK = _CK
    NC = TP // CK
    PAD = K // 2
    H = 16
    SL = _up(M + 2 * H, 32)
    XS = _up(M, 32)
    QS = _up(M, 64)
    NS = D // 128
    NTB = T // M
    NT = B * NTB
    NA = NT // 2
    NP = M // PR
    KP = _up(K, 32)
    NST = NP + 1
    NTAIL = ML // PR + 1
    TLO = M - NTAIL * PR
    eps = 1e-5
    taps = [k for b in range(8) for k in range(b, K, 8)]
    qscale = (D ** -0.5) * math.log2(math.e)
    gc1 = math.sqrt(2.0 / math.pi)
    gc2 = gc1 * 0.044715
    assert T % (2 * M) == 0 and M % PR == 0 and PR % 16 == 0 and ML % PR == 0 and PAD <= H
    assert TP - T < 128 and D % 128 == 0 and NS >= 2 and NT >= 4 and NC >= 2

    def gelu2(h):
        return h * (1.0 + jnp.tanh(h * (gc1 + gc2 * (h * h))))

    def ln(v, e):
        mu = jnp.mean(v, axis=-1, keepdims=True)
        c = v - mu
        var = jnp.mean(c * c, axis=-1, keepdims=True)
        return c * jnp.exp2(jnp.log(var + e) * (-0.5 / math.log(2.0)))

    def kernel(x_hbm, wqkv_hbm, wo_hbm, wmi_hbm, dwc_hbm, wmo_hbm, dwm_hbm, wmg_hbm, out_hbm,
               x_v, o_v, wqkv_v, wo_v, wmo_v, wmg_v, wall, wg, wbc, wbm, k_s, q_s, v_s, u_s,
               g_s, mg_s, ml_s, y_s, kt_s, dwc_v, dwm_v, xsem, wsem, osem):

        def x_copy(t):
            return pltpu.make_async_copy(x_hbm.at[pl.ds(2 * t, 2)],
                                         x_v.at[pl.ds(2 * t, 2), pl.ds(0, M), :], xsem.at[t])

        def h_copy(j):
            return pltpu.make_async_copy(x_hbm.at[j], x_v.at[j, pl.ds(0, M), :],
                                         xsem.at[0 if j == 0 else NA])

        def o_copy(n, lo=0, cnt=M):
            return pltpu.make_async_copy(o_v.at[n, pl.ds(lo, cnt), :],
                                         out_hbm.at[n, pl.ds(lo, cnt), :], osem.at[0])

        wqk_copy = pltpu.make_async_copy(wqkv_hbm.at[:, pl.ds(0, 2 * D)],
                                         wqkv_v.at[:, pl.ds(0, 2 * D)], wsem.at[0])
        wmi_copies = [
            pltpu.make_async_copy(wmi_hbm.at[:, pl.ds(D, D)], wall.at[:, pl.ds(D, D)], wsem.at[1]),
            pltpu.make_async_copy(wmi_hbm.at[:, pl.ds(0, D)], wall.at[:, pl.ds(2 * D, D)], wsem.at[1]),
        ]
        late_copies = [
            pltpu.make_async_copy(wqkv_hbm.at[:, pl.ds(2 * D, D)], wqkv_v.at[:, pl.ds(2 * D, D)],
                                  wsem.at[2]),
            pltpu.make_async_copy(wo_hbm, wo_v, wsem.at[2]),
            pltpu.make_async_copy(dwc_hbm, dwc_v, wsem.at[2]),
            pltpu.make_async_copy(dwm_hbm, dwm_v, wsem.at[2]),
            pltpu.make_async_copy(wmo_hbm, wmo_v, wsem.at[2]),
            pltpu.make_async_copy(wmg_hbm, wmg_v, wsem.at[2]),
        ]
        h_copy(0).start()
        wqk_copy.start()
        for c in wmi_copies:
            c.start()
        h_copy(1).start()

        zh = jnp.zeros((H, 128), _F32)
        for b in range(B):
            first, last = (b * (NTB + 1) + 1) * SL, (b + 1) * (NTB + 1) * SL - SL
            for s in range(NS):
                for arr in (g_s, mg_s, ml_s):
                    arr[s, first:first + H, :] = zh
                    arr[s, last + H + M:last + 2 * H + M, :] = zh
                if TP > T:
                    k_s[b, s, T:TP, :] = jnp.zeros((TP - T, 128), _BF16)
            if TP > T:
                v_s[b, T:TP, :] = jnp.zeros((TP - T, 128), _BF16)
        for s in range(NS):
            mg_s[s, SL + H + M:SL + 2 * H + M, :] = zh

        mods = [NT + 2]

        def fresh(n):
            mods[0] += 1
            if mods[0] & (mods[0] - 1) == 0:
                mods[0] += 1
            return jax.lax.rem(n, mods[0])

        def batch_of(n, per):
            b = 0
            for j in range(1, B):
                b = b + (n >= j * per).astype(jnp.int32)
            return b

        slots = {}

        def slot(n):
            if id(n) not in slots:
                slots[id(n)] = (n, pl.multiple_of((n + batch_of(n, NTB)) * SL, 32))
            return slots[id(n)][1]

        def put(arr, n, lo, val, j=0):
            cnt = val.shape[0]
            base = slot(n)
            s0 = (j + 1) * SL
            for s in range(NS):
                v = val[:, s * 128:(s + 1) * 128]
                arr[s, pl.ds(base + (s0 + H + lo), cnt), :] = v
                if lo == 0:
                    arr[s, pl.ds(base + (s0 - SL + H + M), H), :] = v[0:H]
                if lo + cnt == M:
                    arr[s, pl.ds(base + (s0 + SL), H), :] = v[cnt - H:cnt]

        def krow_of(t):
            b = batch_of(t, NA // B)
            return b, pl.multiple_of((t - b * (NA // B)) * (2 * M), 16)

        def a1(t, js=(0, 1)):
            b, krow = krow_of(t)
            lo, cnt = js[0] * M, len(js) * M
            x = jnp.concatenate([x_v[2 * t + j, 0:M, :] for j in js], axis=0)
            xa = ln(x.astype(_F32), eps)
            for s in range(NS):
                k_s[b, s, pl.ds(krow + lo, cnt), :] = xa[:, s * 128:(s + 1) * 128].astype(_BF16)
            lane = jax.lax.broadcasted_iota(jnp.int32, (cnt, 128), 1)
            v_s[b, pl.ds(krow + lo, cnt), :] = jnp.where(lane == 127, 1.0, xa[:, D - 128:]).astype(_BF16)

        def a2(t, js=(0, 1)):
            b, krow = krow_of(t)
            lo, cnt = js[0] * M, len(js) * M
            xa = jnp.concatenate([k_s[b, s, pl.ds(krow + lo, cnt), :] for s in range(NS)], axis=1)
            y = jnp.dot(xa, wall[...], preferred_element_type=_F32)
            g = ln(gelu2(y[:, D:2 * D]), 4.0 * eps)
            n0 = 2 * t
            for j in js:
                rows = slice(j * M - lo, (j + 1) * M - lo)
                u_s[2 * t + j] = y[rows, 2 * D:3 * D]
                put(g_s, n0, 0, g[rows], j)
                for s in range(NS):
                    q_s[2 * t + j, s, 0:M, :] = y[rows, s * 128:(s + 1) * 128].astype(_BF16)

        def late_prep():
            for b in range(B):
                k0 = jnp.concatenate([k_s[b, s, 0:CK, :] for s in range(NS)], axis=1)
                kt_s[b] = k0.astype(_F32).T.astype(_BF16)
            wvo = jnp.dot(wqkv_v[:, 2 * D:3 * D], wo_v[...], preferred_element_type=_F32)
            wg[...] = (wvo - wvo[D - 1:D, :]).astype(_BF16)
            dwc = dwc_v[...].astype(_F32) * 0.5
            dwm = dwm_v[...].astype(_F32)
            for k in range(K):
                for s in range(NS):
                    wbc[s, k] = jnp.broadcast_to(dwc[k:k + 1, s * 128:(s + 1) * 128], (8, 128))
                for s in range(2 * NS):
                    w = dwm[k:k + 1, s * 128:(s + 1) * 128]
                    if k == PAD:
                        w = w + 1.0
                    wbm[s, k] = jnp.broadcast_to(w, (8, 128))

        def steps(*fns):
            def step(i, carry):
                for j, fn in enumerate(fns):
                    pl.when(i == j)(lambda j=j, fn=fn: fn(i - j))
                return carry
            jax.lax.fori_loop(0, len(fns), step, 0)

        def start0(z):
            h_copy(0).wait()
            x_copy(1).start()
            a1(fresh(z), (0,))
            wqk_copy.wait()
            a = jax.lax.dot_general(wqkv_v[:, 0:D], wqkv_v[:, D:2 * D], _NT,
                                    preferred_element_type=_F32)
            wall[:, 0:D] = (a * qscale).astype(_BF16)

        def start1(z):
            for c in wmi_copies:
                c.wait()
            h_copy(1).wait()
            a2(fresh(z), (0,))
            a1(fresh(z), (1,))

        def start2(z):
            x_copy(1).wait()
            for t in range(2, NA):
                x_copy(t).start()
            for c in late_copies:
                c.start()
            a2(fresh(z), (1,))
            a1(fresh(z + 1))

        def phase_a(t, carry):
            x_copy(t + 1).wait()
            a2(t)
            a1(fresh(t + 1))
            return carry

        def last_a(z):
            for c in late_copies:
                c.wait()
            a2(fresh(z + (NA - 1)))
            late_prep()

        def conv(src, wb, ws, n, o):
            base = slot(n)
            outs = []
            for s in range(NS):
                acc = None
                for k in taps:
                    xk = src[s, pl.ds(base + (SL + o + H + k - PAD), PR), :].reshape(PR // 8, 8, 128)
                    term = xk * wb[ws + s, k][None]
                    acc = term if acc is None else acc + term
                outs.append(acc.reshape(PR, 128))
            return jnp.concatenate(outs, axis=1)

        def loc_piece(n, o):
            def run():
                z = (gelu2(u_s[n, o:o + PR, :]) * conv(g_s, wbc, 0, n, o)).astype(_BF16)
                put(ml_s, n, o, jnp.dot(z, wmo_v[...], preferred_element_type=_F32))
            return run

        def merge_loc(n, o):
            m = conv(ml_s, wbm, NS, n, o).astype(_BF16)
            return (x_v[n, o:o + PR, :].astype(_F32)
                    + jnp.dot(m, wmg_v[D:2 * D, :], preferred_element_type=_F32))

        def merge_glob(n, o, y1):
            m = conv(mg_s, wbm, 0, n, o).astype(_BF16)
            y = y1 + jnp.dot(m, wmg_v[0:D, :], preferred_element_type=_F32)
            o_v[n, o:o + PR, :] = y.astype(_BF16)

        def locs(n):
            slot(n)
            return [loc_piece(n, r * PR) for r in range(NP)]

        def merges(n):
            n2 = jnp.maximum(n - 2, 0)
            n1 = n - 1
            slot(n2)
            slot(n1)
            out = []
            for (nn, o) in [(n2, M - PR)] + [(n1, r * PR) for r in range(NP - 1)]:
                def two(nn=nn, o=o):
                    st = []
                    return [lambda: st.append(merge_loc(nn, o)), lambda: merge_glob(nn, o, st[0])]
                out += two()
            return out

        def end_loc(n, i):
            nn, o = (n - 1, M - PR) if i == 0 else (n, (i - 1) * PR)
            slot(nn)
            return nn, o

        def stash(n, i):
            nn, o = end_loc(n, i)

            def run():
                y_s[i] = merge_loc(nn, o)
            return run

        def finish(n, i):
            nn, o = end_loc(n, i)
            return lambda: merge_glob(nn, o, y_s[i])

        def attend(n, b, off, mr, pieces):
            hooks = {}
            cnt = len(pieces)
            for i, pc in enumerate(pieces):
                if cnt == 2 * NC - 1:
                    h = i + 1
                else:
                    done = lambda h: min(h // 2 + 2, NC) + (h + 1) // 2
                    want = (i + 3) * (2 * NC) / (cnt + 2)
                    h = min((h for h in range(2 * NC) if h != 2 * NC - 2),
                            key=lambda h: abs(done(h) - want))
                hooks.setdefault(h, []).append(pc)

            q = jnp.concatenate([q_s[n, s, off:off + mr, :] for s in range(NS)], axis=1)

            def qk(c):
                if c == 0:
                    return jnp.dot(q, kt_s[b], preferred_element_type=_F32)
                kk = jnp.concatenate([k_s[b, s, c * CK:(c + 1) * CK, :] for s in range(NS)], axis=1)
                s = jax.lax.dot_general(q, kk, _NT, preferred_element_type=_F32)
                if c == NC - 1 and TP > T:
                    lane = jax.lax.broadcasted_iota(jnp.int32, (mr, 128), 1)
                    s_last = jnp.where(lane < T - (TP - 128), s[:, CK - 128:], -jnp.inf)
                    s = jnp.concatenate([s[:, :CK - 128], s_last], axis=1)
                return s

            s_next = qk(0)
            for c in range(NC):
                s = s_next
                if c + 1 < NC:
                    s_next = qk(c + 1)
                for hk in hooks.get(2 * c, []):
                    hk()
                m_c = jnp.max(s, axis=1, keepdims=True)
                if c == 0:
                    m_new = m_c
                else:
                    m_new = jnp.maximum(m_run, m_c)
                    alpha = jnp.exp2(m_run - m_new)
                pr = jnp.exp2(s - m_new)
                vv = jnp.concatenate([k_s[b, s_, c * CK:(c + 1) * CK, :] for s_ in range(NS - 1)]
                                     + [v_s[b, c * CK:(c + 1) * CK, :]], axis=1)
                pv = jnp.dot(pr.astype(_BF16), vv, preferred_element_type=_F32)
                acc = pv if c == 0 else acc * alpha + pv
                m_run = m_new
                for hk in hooks.get(2 * c + 1, []):
                    hk()
            glob = jnp.dot(acc.astype(_BF16), wg[...], preferred_element_type=_F32)
            put(mg_s, n, off, glob * (1.0 / acc[:, D - 1:D]))

        def first_b(z):
            n = fresh(z)
            attend(n, 0, 0, M, locs(n) + locs(n + 1))

        def phase_b(i, carry):
            n = fresh(i)
            attend(n, batch_of(i, NTB), 0, M, merges(n) + locs(n + 1))

            @pl.when(i >= 2)
            def _():
                o_copy(i - 2).start()
            return carry

        def end0(z):
            n = fresh(z + (NT - 1))
            attend(n, B - 1, 0, M - ML, merges(n) + [stash(n, j) for j in range(NST)])
            o_copy(NT - 3).start()

        def end1(z):
            n = fresh(z + (NT - 1))
            attend(n, B - 1, M - ML, ML, [finish(n, j) for j in range(NST - NTAIL)])
            o_copy(NT - 2).start()
            o_copy(NT - 1, 0, TLO).start()

        def end2(z):
            n = fresh(z + (NT - 1))
            for j in range(NTAIL):
                finish(n, NST - NTAIL + j)()
                o_copy(NT - 1, TLO + j * PR, PR).start()

        steps(start0, start1, start2)
        jax.lax.fori_loop(1, NA - 1, phase_a, 0)
        steps(last_a, first_b)
        jax.lax.fori_loop(1, NT - 1, phase_b, 0)
        steps(end0, end1, end2)

        for i in range(NT - 1):
            o_copy(i).wait()
        o_copy(NT - 1, 0, TLO).wait()
        for i in range(NTAIL):
            o_copy(NT - 1, TLO + i * PR, PR).wait()

    scratch = [
        pltpu.VMEM((NT, XS, D), _BF16),
        pltpu.VMEM((NT, XS, D), _BF16),
        pltpu.VMEM((D, 3 * D), _BF16),
        pltpu.VMEM((D, D), _BF16),
        pltpu.VMEM((D, D), _BF16),
        pltpu.VMEM((2 * D, D), _BF16),
        pltpu.VMEM((D, 3 * D), _BF16),
        pltpu.VMEM((D, D), _BF16),
        pltpu.VMEM((NS, KP, 8, 128), _F32),
        pltpu.VMEM((2 * NS, KP, 8, 128), _F32),
        pltpu.VMEM((B, NS, TP, 128), _BF16),
        pltpu.VMEM((NT, NS, QS, 128), _BF16),
        pltpu.VMEM((B, TP, 128), _BF16),
        pltpu.VMEM((NT, M, D), _F32),
        pltpu.VMEM((NS, (NT + B + 1) * SL, 128), _F32),
        pltpu.VMEM((NS, (NT + B + 1) * SL, 128), _F32),
        pltpu.VMEM((NS, (NT + B + 1) * SL, 128), _F32),
        pltpu.VMEM((NST, PR, D), _F32),
        pltpu.VMEM((B, D, CK), _BF16),
        pltpu.VMEM((K, D), _BF16),
        pltpu.VMEM((K, 2 * D), _BF16),
        pltpu.SemaphoreType.DMA((NA + 1,)),
        pltpu.SemaphoreType.DMA((3,)),
        pltpu.SemaphoreType.DMA((1,)),
    ]
    return kernel, scratch, NT


@jax.jit
def pallas_standalone__conformer_family_e_branchformer__speech_kernel(
    x: jax.Array,
    w_qkv: jax.Array,
    w_att_out: jax.Array,
    w_mlp_in: jax.Array,
    dw_csgu: jax.Array,
    w_mlp_out: jax.Array,
    dw_merge: jax.Array,
    w_merge: jax.Array,
):
    B, T, D = x.shape
    K = dw_csgu.shape[0]
    kernel, scratch, NT = _make_kernel(B, T, D, K)
    out = pl.pallas_call(
        kernel,
        out_shape=jax.ShapeDtypeStruct((NT, _M, D), x.dtype),
        in_specs=[pl.BlockSpec(memory_space=pl.ANY)] * 8,
        out_specs=pl.BlockSpec(memory_space=pl.ANY),
        scratch_shapes=scratch,
        compiler_params=pltpu.CompilerParams(vmem_limit_bytes=110 * 1024 * 1024),
    )(x.reshape(NT, _M, D), w_qkv, w_att_out, w_mlp_in, dw_csgu, w_mlp_out, dw_merge, w_merge)
    return out.reshape(B, T, D)
```
